```python
import os as _os
_os.environ.setdefault("JAX_PLATFORMS", "cpu")
import jax
import jax.numpy as jnp

def _softmax(x, axis=-1):
    return jax.nn.softmax(x, axis=axis)
def _gelu(x):
    return jax.nn.gelu(x, approximate=True)
def _silu(x):
    return jax.nn.silu(x)
def _sigmoid(x):
    return jax.nn.sigmoid(x)
def _layernorm(x, axis=-1, eps=1e-5):
    m = jnp.mean(x, axis=axis, keepdims=True)
    v = jnp.var(x, axis=axis, keepdims=True)
    return (x - m) / jnp.sqrt(v + eps)
def _scatter_add(tgt, idx, src, axis=0):
    return tgt.at[idx].add(src)
def _segment_sum(src, seg, n):
    return jax.ops.segment_sum(src, seg, n)
class _Rng:
    def __init__(self, key):
        self._k = key
    def _next(self):
        self._k, sub = jax.random.split(self._k)
        return sub
    def normal(self, shape):
        return jax.random.normal(self._next(), shape, dtype=jnp.bfloat16)
    def randint(self, lo, hi, shape):
        return jax.random.randint(self._next(), shape, lo, hi, dtype=jnp.int32)
    def uniform(self, shape, lo=0.0, hi=1.0):
        return jax.random.uniform(self._next(), shape, jnp.bfloat16, lo, hi)
    def permutation(self, n):
        return jax.random.permutation(self._next(), n)


kernel_name = 'parallel_sum__sliding_local_dilated__geglu_ffn__prompt'

def setup_inputs():
    _rng = _Rng(jax.random.key(int.from_bytes(__import__("os").urandom(4), "little")))
    _w = (lambda a: (lambda t: t.astype(jnp.bfloat16) if jnp.issubdtype(t.dtype, jnp.floating) else t)(jnp.asarray(a)))
    def _A_setup():
        B, S, D = 1, 2048, 640
        return {
            "x": _w((lambda *s: _rng.normal(s) * 0.05)(B, S, D)),
            "wqkv": _w((lambda *s: _rng.normal(s) * 0.05)(D, 3 * D)),
            "wo": _w((lambda *s: _rng.normal(s) * 0.05)(D, D)),
        }
    _A_in = _A_setup()

    def _B_setup():
        B, S, D, F = 1, 2048, 640, 1728
        return {
            "x": _w((lambda *s: _rng.normal(s) * 0.05)(B, S, D)),
            "w_gate": _w((lambda *s: _rng.normal(s) * 0.05)(D, F)),
            "w_up": _w((lambda *s: _rng.normal(s) * 0.05)(D, F)),
            "w_down": _w((lambda *s: _rng.normal(s) * 0.05)(F, D)),
        }
    _B_in = _B_setup()

    return {
        "A_x": _A_in["x"],
        "A_wqkv": _A_in["wqkv"],
        "A_wo": _A_in["wo"],
        "B_x": _B_in["x"],
        "B_w_gate": _B_in["w_gate"],
        "B_w_up": _B_in["w_up"],
        "B_w_down": _B_in["w_down"],
    }

def reference(A_x, A_wqkv, A_wo, B_x, B_w_gate, B_w_up, B_w_down):
    def _A_ref(x, wqkv, wo):
        B, S, D = x.shape
        H = 32; Dh = D // H
        W, dil = 8, 2
        qkv = (lambda x, *d: x.transpose(*d))((x @ wqkv).reshape(B, S, 3, H, Dh), 2, 0, 3, 1, 4)
        q, k, v = qkv[0], qkv[1], qkv[2]
        scale = Dh ** -0.5
        pos = jnp.arange(S)
        off = jnp.arange(W) * dil
        idx = pos[:, None] - off[None, :]
        mask = idx >= 0
        idx_c = jnp.where(mask, idx, 0).reshape(-1)
        kg = k[:, :, idx_c, :].reshape(B, H, S, W, Dh)
        vg = v[:, :, idx_c, :].reshape(B, H, S, W, Dh)
        logits = jnp.einsum("bhsd,bhswd->bhsw", q, kg) * scale
        logits = jnp.where(mask[None, None, :, :], logits, -1e9)
        attn = _softmax(logits, axis=-1)
        o = jnp.einsum("bhsw,bhswd->bhsd", attn, vg)
        return (lambda x, *d: x.transpose(*d))(o, 0, 2, 1, 3).reshape(B, S, D) @ wo

    def _B_ref(x, w_gate, w_up, w_down):
        return (_gelu(x @ w_gate) * (x @ w_up)) @ w_down

    x = A_x
    xn = _layernorm(x, axis=-1)
    return x + _A_ref(xn, A_wqkv, A_wo) + _B_ref(xn, B_w_gate, B_w_up, B_w_down)
```

```python
import functools
import math
import jax
import jax.numpy as jnp
import jax.experimental.pallas as pl
import jax.experimental.pallas.tpu as pltpu

S, D, F = 2048, 640, 1728
H, DH, W, DIL = 32, 20, 8, 2
HALO = 16
L = 128
NT = D // L
NJ = 7
FM = (F // L) * L
f32, bf16 = jnp.float32, jnp.bfloat16


def _dot(a, b):
    return jnp.dot(a, b, preferred_element_type=f32)


def _dot_nt(a, b):
    return jax.lax.dot_general(a, b, (((1,), (1,)), ((), ())), preferred_element_type=f32)


def _geglu(g, u):
    c = math.sqrt(2.0 / math.pi)
    t = jnp.tanh(g * (c + (c * 0.044715) * (g * g)))
    hg = 0.5 * g
    return (hg + hg * t) * u


def _lhs_terms(a11, a12, a21, a22):
    return [a11 + a22, a21 + a22, a11, a22, a11 + a12, a21 - a11, a12 - a22]


def _rhs_terms(b11, b12, b21, b22):
    return [b11 + b22, b11, b12 - b22, b21 - b11, b22, b11 + b12, b21 + b22]


def _combine(m):
    return m[0] + m[3] - m[4] + m[6], m[2] + m[4], m[1] + m[3], m[0] - m[1] + m[2] + m[5]


def _put(ref, idx, r0, val, e0=0):
    n = val.shape[0]
    r = r0 if isinstance(r0, int) else pl.multiple_of(r0, n)
    for e in range(val.shape[1] // L):
        ref[idx + (e0 + e, pl.ds(r, n), slice(None))] = val[:, e * L:(e + 1) * L].astype(bf16)


def _get(ref, idx, n):
    return jnp.concatenate([ref[idx + (e,)] for e in range(n)], axis=1)


def _grid(rows):
    return jnp.concatenate([jnp.concatenate(r, axis=1) for r in rows], axis=0)


def _mix(a, b):
    keyed = [((i + 0.5) / len(a), t) for i, t in enumerate(a)] + [((i + 0.5) / len(b), t) for i, t in enumerate(b)]
    return [t for _, t in sorted(keyed, key=lambda kt: kt[0])]


class _Tasks:
    def __init__(self, tasks, slots, skip=0):
        self.tasks, self.slots, self.skip, self.n, self.done = list(tasks), slots, skip, 0, 0

    def tick(self, val=None):
        self.n += 1
        want = -(-len(self.tasks) * max(0, self.n - self.skip) // self.slots)
        while self.done < min(want, len(self.tasks)):
            self.tasks[self.done](val)
            self.done += 1

    def flush(self):
        for t in self.tasks[self.done:]:
            t(None)
        self.done = len(self.tasks)


SUMS = (0, 2, 3, 5, 6)
_GU = lambda j, n, kt, e: ((j * 5 + n) * 2 + kt) * 2 + e
_QC = lambda p, i, kt, e: ((p * 7 + i) * 2 + kt) * 2 + e
_QK = lambda p, c: _QC(4, 0, 0, 0) + p * 4 + c
_Q4 = lambda p, kt: _QK(3, 0) + p * NT + kt
_OC = lambda i, kt, e: _Q4(3, 0) + (i * 2 + kt) * 2 + e
_OK = lambda c: _OC(7, 0, 0) + c
_O4 = lambda kt: _OK(4) + kt
_DC = lambda n, e: _O4(NT) + (n * 2 + e) * NJ
NW = _DC(5, 0)


def build(tm=256, ar=16, lnr=16, sr=32, ska=0, flags=None, sa=50, sp=14, sb=(1, 20), sl=(1, 14), scope=False):
    nb = S // tm
    hm = tm // 2
    npro = 2
    wrows = 160

    def kernel(x_hbm, wqkv_hbm, wo_hbm, wg_hbm, wu_hbm, wd_hbm, o_hbm,
               x_s, xc_s, gu_r, qkv_r, wo_r, wd_r, w_s, g_s, tmp_s, a_s, kv_s, hc_s, ac_s, z_s, o_s, xsem, gsem, wsem, osem):
        def x_copy(b):
            return pltpu.make_async_copy(x_hbm.at[pl.ds(b * tm, tm)], x_s.at[b], xsem.at[b])

        def gu_copies(j):
            if j < NJ - 1:
                parts = [(wg_hbm, j * L, L, 0), (wu_hbm, j * L, L, L),
                         (wg_hbm, (j + NJ) * L, L, 2 * L), (wu_hbm, (j + NJ) * L, L, 3 * L)]
            else:
                parts = [(wg_hbm, j * L, L, 0), (wg_hbm, FM, F - FM, L), (wu_hbm, FM, F - FM, L + F - FM),
                         (wu_hbm, j * L, L, 2 * L), (wu_hbm, j * L, L, 3 * L)]
            return [pltpu.make_async_copy(src.at[pl.ds(r, n)], gu_r.at[j, pl.ds(o, n)], gsem.at[j])
                    for src, r, n, o in parts]

        def gu_wait(j):
            pltpu.make_async_copy(gu_r.at[j], gu_r.at[j], gsem.at[j]).wait()

        qkv_copies = [pltpu.make_async_copy(wqkv_hbm.at[:, pl.ds(p * D, D)], qkv_r.at[p], wsem.at[p]) for p in range(3)]
        wo_copy = pltpu.make_async_copy(wo_hbm, wo_r.at[0], wsem.at[3])
        wd_copies = [pltpu.make_async_copy(wd_hbm.at[pl.ds(0, NJ * L)], wd_r.at[0], wsem.at[4]),
                     pltpu.make_async_copy(wd_hbm.at[pl.ds(NJ * L, F - NJ * L)], wd_r.at[1, pl.ds(0, F - NJ * L)], wsem.at[5])]

        def o_copy(b):
            return pltpu.make_async_copy(o_s.at[b], o_hbm.at[pl.ds(pl.multiple_of(b * tm, tm), tm)], osem.at[b])

        def mark(name, fn):
            if scope:
                with jax.named_scope("z_" + name):
                    fn()
            else:
                fn()

        def wtile(t):
            return w_s[pl.ds(t * L if isinstance(t, int) else pl.multiple_of(t * L, L), L), :]

        def set_wtile(t, val, r=0):
            n = val.shape[0]
            w_s[pl.ds(t * L + r if isinstance(t, int) else pl.multiple_of(t * L + r, n), n), :] = val.astype(bf16)

        def after(ref, spare, fn, *args):
            def task(val):
                if val is not None:
                    ref[spare + z_s[0], 0:16, 0:L] = val[-16:, -L:].astype(ref.dtype)
                fn(*args)

            return task

        def ln_tasks(b):
            dst = b
            src = b if isinstance(b, int) else jnp.minimum(b, nb - 1)

            def norm(r):
                x = x_s[src, r:r + lnr, :].astype(f32)
                xc = x - jnp.sum(x, axis=-1, keepdims=True) * (1.0 / D)
                v = jnp.sum(xc * xc, axis=-1, keepdims=True) * (1.0 / D)
                return xc * jax.lax.rsqrt(v + 1e-5)

            def piece(r):
                y1, y2 = norm(r), norm(hm + r)
                a12, a21 = y1[:, 2 * L:4 * L], y2[:, 0:2 * L]
                last = jnp.concatenate([y1[:, 4 * L:], y2[:, 4 * L:]], axis=1)
                for i, t in enumerate(_lhs_terms(y1[:, 0:2 * L], a12, a21, y2[:, 2 * L:4 * L]) + [a12, a21, last]):
                    _put(xc_s, (dst, i), r, t)

            return [after(x_s, nb, piece, r) for r in range(0, hm, lnr)]

        def full_rows(ref, idx):
            g = lambda i, e: ref[idx + (i, e)]
            return _grid([[g(2, 0), g(2, 1), g(7, 0), g(7, 1), g(9, 0)], [g(8, 0), g(8, 1), g(3, 0), g(3, 1), g(9, 1)]])

        def project(b, wc, wk, tick):
            ms = []
            for i in range(7):
                ms.append(_dot_nt(_get(xc_s, (b, i), 2), wc(i)))
                tick(ms[-1])
            r = _dot_nt(jnp.concatenate([xc_s[b, 9, 0], xc_s[b, 9, 1]], axis=0), wk())
            tick(r)
            n = r.shape[1] // 2
            c11, c12, c21, c22 = _combine(ms)
            return c11 + r[:hm, :n], c12 + r[:hm, n:], c21 + r[hm:, :n], c22 + r[hm:, n:]

        def gu_tasks(j, z):
            def piece(kt, e, r):
                t = lambda n, k: gu_r[j, (2 * n + e) * L + r:(2 * n + e) * L + r + H, k * L:(k + 1) * L].astype(f32)
                terms = _rhs_terms(t(0, kt), t(1, kt), t(0, kt + 2), t(1, kt + 2))
                for n, i in enumerate(SUMS):
                    g_s[_GU(j, n, kt, e) + z, r:r + H, :] = terms[i].astype(bf16)

            return [lambda _, a=(kt, e, r): piece(*a) for kt in range(2) for e in range(2) for r in range(0, L, H)]

        def gu_weights(j, ne):
            def wc(i):
                if i == 1:
                    return gu_r[j, 0:ne * L, 0:2 * L]
                if i == 4:
                    return gu_r[j, 2 * L:(2 + ne) * L, 2 * L:4 * L]
                return _grid([[g_s[_GU(j, SUMS.index(i), kt, e)] for kt in range(2)] for e in range(ne)])

            return wc

        def store_h(b, j, h11, h12, h21, h22):
            for i, t in enumerate(_lhs_terms(h11, h12, h21, h22) + [h12, h21]):
                _put(hc_s, (b, i), 0, t, j)

        def gate_up(b, j, tick):
            cs = project(b, gu_weights(j, 2), lambda: gu_r[j, :, 4 * L:], tick)
            store_h(b, j, *[_geglu(c[:, :L], c[:, L:]) for c in cs])

        def gate_up_last(b, tick):
            j = NJ - 1
            r = _dot_nt(full_rows(xc_s, (b,)), gu_r[j, L:2 * L, :])
            lane = jax.lax.broadcasted_iota(jnp.int32, (tm, L), 1)
            ht = jnp.where(lane < F - FM, _geglu(r, pltpu.roll(r, L // 2, 1)), 0.0)
            wk = lambda: jnp.concatenate([gu_r[j, 0:L, 4 * L:], gu_r[j, 2 * L:3 * L, 4 * L:]], axis=0)
            g1, u1, g2, u2 = project(b, gu_weights(j, 1), wk, tick)
            store_h(b, j, _geglu(g1, u1), ht[:hm], _geglu(g2, u2), ht[hm:])

        def perm_tile(slab, c):
            return jnp.concatenate([tmp_s[slab, pl.ds(4 * c + e, H, stride=DH), :] for e in range(4)], axis=0)

        def perm_rows(slab, c, d):
            return tmp_s[slab, pl.ds(4 * c + d, H, stride=DH), :]

        def qkv_tasks(p, kt):
            def load(slab, k, c):
                rows = pl.ds(pl.multiple_of(k * L, L), L)
                tmp_s[slab, c * L:(c + 1) * L, :] = qkv_r[p, rows, c * L:(c + 1) * L].astype(f32).T

            def sums(e, d):
                terms = _rhs_terms(perm_rows(0, e, d), perm_rows(0, 2 + e, d), perm_rows(1, e, d), perm_rows(1, 2 + e, d))
                for i, t in enumerate(terms):
                    set_wtile(_QC(p, i, kt, e), t, d * H)

            def copy(t, slab, c):
                set_wtile(t, perm_tile(slab, c))

            P = functools.partial(after, tmp_s, NT)
            return ([after(qkv_r, 3, load, s, k, c) for s, k in enumerate((kt, kt + 2, 4)) for c in range(NT)],
                    [P(copy, _Q4(p, kt), 0, 4), P(copy, _Q4(p, kt + 2), 1, 4)]
                    + [P(sums, e, d) for e in range(2) for d in range(4)]
                    + [P(copy, _Q4(p, 4), 2, 4)] + [P(copy, _QK(p, c), 2, c) for c in range(4)])

        def wd_tasks(r0):
            def piece(r, n, e):
                t = lambda k, c: wd_r[k, pl.ds(pl.multiple_of(r, 16), n), c * L:(c + 1) * L].astype(f32)
                terms = _rhs_terms(t(0, e), t(0, 2 + e), t(1, e), t(1, 2 + e))
                for m, i in enumerate(SUMS):
                    w_s[pl.ds(pl.multiple_of(_DC(m, e) * L + r, 16), n), :] = terms[i].astype(bf16)

            return [after(wd_r, 2, piece, r0 + r, H, e) for r in range(0, wrows, H) for e in range(2)]

        def mid_tasks():
            def qk4(kt, r):
                t = lambda p, k: w_s[_Q4(p, k) * L + r:_Q4(p, k) * L + r + H, :].astype(f32)
                for i, v in enumerate(_rhs_terms(t(0, kt), t(1, kt), t(0, kt + 2), t(1, kt + 2))):
                    set_wtile(_QC(3, i, kt, 0), v, r)

            def load(c):
                tmp_s[c] = wo_r[0, :, c * L:(c + 1) * L].astype(f32)

            def sums(kt, e, d):
                terms = _rhs_terms(perm_rows(e, kt, d), perm_rows(2 + e, kt, d), perm_rows(e, kt + 2, d), perm_rows(2 + e, kt + 2, d))
                for i, t in enumerate(terms):
                    set_wtile(_OC(i, kt, e), t, d * H)

            def copy(t, slab, c):
                set_wtile(t, perm_tile(slab, c))

            P = functools.partial(after, tmp_s, NT)
            return ([lambda _, a=(kt, r): qk4(*a) for kt in range(2) for r in range(0, L, H)] + [after(wo_r, 1, load, c) for c in range(NT)]
                    + [P(sums, kt, e, d) for kt in range(2) for e in range(2) for d in range(4)]
                    + [P(copy, _OK(c), c, 4) for c in range(4)] + [P(copy, _O4(kt), 4, kt) for kt in range(NT)])

        def qkv(b, slot, tick, tock):
            def put(p, c, r0, val):
                if p == 0:
                    a_s[slot + c, r0:r0 + val.shape[0], :] = val
                else:
                    kv_s[2 * slot + (p - 1) * NT + c, HALO + r0:HALO + r0 + val.shape[0], :] = val

            for p in range(3):
                wc = lambda i: _grid([[wtile(_QC(p, i, kt, e)) for kt in range(2)] for e in range(2)])
                wk = lambda: _grid([[wtile(_QK(p, c))] for c in range(4)])
                for n, cv in enumerate(project(b, wc, wk, tick)):
                    for e in range(2):
                        put(p, 2 * (n % 2) + e, hm * (n // 2), cv[:, e * L:(e + 1) * L])
                tock()
            wc = lambda i: _grid([[wtile(_QC(3, i, kt, 0)) for kt in range(2)]])
            wk = lambda: _grid([[wtile(_Q4(p, 4))] for p in range(2)])
            for n, cv in enumerate(project(b, wc, wk, tick)):
                put(n % 2, 4, hm * (n // 2), cv)
            tock()
            put(2, 4, 0, _dot_nt(full_rows(xc_s, (b,)), _grid([[wtile(_Q4(2, kt)) for kt in range(NT)]])))

        def attention(b, slot, r):
            q = [a_s[slot + c, r:r + ar, :] for c in range(NT)]
            ls = []
            for w in range(W):
                o = HALO + r - DIL * w
                s = q[0] * kv_s[2 * slot, o:o + ar, :]
                for c in range(1, NT):
                    s = s + q[c] * kv_s[2 * slot + c, o:o + ar, :]
                s = s + pltpu.roll(s, 2 * H, 1)
                s = s + pltpu.roll(s, H, 1)
                if r < DIL * w:
                    row = jax.lax.broadcasted_iota(jnp.int32, (ar, L), 0) + (r + b * tm)
                    s = jnp.where(row >= DIL * w, s, -1e9 * math.sqrt(DH))
                ls.append(s)
            m = functools.reduce(jnp.maximum, ls)
            es = [jnp.exp2((s - m) * (math.log2(math.e) / math.sqrt(DH))) for s in ls]
            inv = 1.0 / functools.reduce(jnp.add, es)
            out = []
            for c in range(NT):
                acc = None
                for w in range(W):
                    o = HALO + r - DIL * w
                    t = es[w] * kv_s[2 * slot + NT + c, o:o + ar, :]
                    acc = t if acc is None else acc + t
                out.append(acc * inv)
            return out

        def attention_pair(b, slot, r):
            o1, o2 = attention(b, slot, r), attention(b, slot, hm + r)
            for e in range(2):
                for i, t in enumerate(_lhs_terms(o1[e], o1[2 + e], o2[e], o2[2 + e]) + [o1[2 + e], o2[e], (o1, o2)[e][4]]):
                    _put(ac_s, (i,), r, t, e)

        def phase_b(b, has_next):
            z = z_s[0]
            slot = (b % 2) * NT + z
            nslot = NT - slot
            if has_next:
                for c in range(2 * NT):
                    kv_s[2 * nslot + c, 0:HALO, :] = kv_s[2 * slot + c, tm:tm + HALO, :]
            first, slots = sb if has_next else sl
            att = [lambda _, r=r: attention_pair(b, slot, r) for r in range(0, hm, ar)]
            for t in att[:first]:
                t(None)
            side = _Tasks(att[first:], slots)
            acc = 2 * NT + z_s[1]
            hcat = lambda i: _get(hc_s, (b, i), NJ)
            for i in range(7):
                for e in range(2):
                    if i == 1:
                        w = wd_r[0, :, e * L:(e + 1) * L]
                    elif i == 4:
                        w = wd_r[1, :, (2 + e) * L:(3 + e) * L]
                    else:
                        w = w_s[_DC(SUMS.index(i), e) * L:(_DC(SUMS.index(i), e) + NJ) * L, :]
                    a_s[acc + i, e * hm:(e + 1) * hm, :] = _dot(hcat(i), w)
                    side.tick()
            a_s[acc + 7, 0:tm, :] = _dot(_grid([[hcat(2), hcat(7)], [hcat(8), hcat(3)]]), _grid([[wd_r[0, :, 4 * L:]], [wd_r[1, :, 4 * L:]]]))
            side.tick()
            if has_next:
                def tock():
                    for _ in range(4):
                        side.tick()

                qkv(b + 1, nslot, lambda _: None, tock)
            side.flush()
            r = _dot(jnp.concatenate([ac_s[9, 0], ac_s[9, 1]], axis=0), _grid([[wtile(_OK(c)) for c in range(4)]]))
            ms = [jnp.concatenate([a_s[acc + i, 0:hm, :], a_s[acc + i, hm:tm, :]], axis=1)
                  + _dot(_get(ac_s, (i,), 2), _grid([[wtile(_OC(i, kt, e)) for e in range(2)] for kt in range(2)]))
                  for i in range(7)]
            for n, cv in enumerate(_combine(ms)):
                rs, cl = slice(hm * (n // 2), hm * (n // 2 + 1)), slice(2 * L * (n % 2), 2 * L * (n % 2 + 1))
                o_s[b, rs, cl] = (x_s[b, rs, cl].astype(f32) + r[rs, cl] + cv).astype(o_s.dtype)
            y4 = a_s[acc + 7, 0:tm, :] + _dot(full_rows(ac_s, ()), w_s[_O4(0) * L:_O4(NT) * L, :])
            o_s[b, :, 4 * L:] = (x_s[b, :, 4 * L:].astype(f32) + y4).astype(o_s.dtype)
            mark("o", o_copy(b).start)

        def start(copies):
            for cp in copies:
                cp.start()

        start([x_copy(0)] + gu_copies(0) + [x_copy(1)])
        z_s[0] = 0
        z_s[1] = 0
        wd_r[1, F - NJ * L:, :] = jnp.zeros((2 * NJ * L - F, D), bf16)
        mark("x", x_copy(0).wait)
        start(gu_copies(1))
        _Tasks(ln_tasks(0), 1).flush()
        mark("g", lambda: gu_wait(0))
        start(gu_copies(2))
        _Tasks(gu_tasks(0, 0), 1).flush()
        mark("x", x_copy(1).wait)
        _Tasks(ln_tasks(1), 1).flush()
        later = [gu_copies(3) + gu_copies(4), gu_copies(5) + [x_copy(2)], gu_copies(6) + qkv_copies[:1],
                 wd_copies, [x_copy(3)] + qkv_copies[1:], [wo_copy]]

        def prologue(j, _):
            mark("g", lambda: gu_wait(j + 1))
            for n, copies in enumerate(later):
                pl.when(j == n)(functools.partial(start, copies))
            side = _Tasks(gu_tasks(j + 1, z_s[0]), sp)
            for b in range(npro):
                gate_up(b, j, side.tick)
            side.flush()

        jax.lax.fori_loop(0, NJ - 1, prologue, None)
        start([x_copy(b) for b in range(4, nb)])
        mark("x", x_copy(npro).wait)
        side = _Tasks(ln_tasks(npro), 14)
        for b in range(npro):
            gate_up_last(b, side.tick)
        side.flush()
        mark("q", qkv_copies[0].wait)
        for cp in wd_copies:
            mark("d", cp.wait)

        def phase_a(b, _):
            t = b - npro
            pl.when(b + 1 < nb)(lambda: mark("a", x_copy(b + 1).wait))
            for p in (1, 2):
                pl.when(t == 2 * p)(qkv_copies[p].wait)
            ln = ln_tasks(b + 1)
            loads, sums = qkv_tasks(t // 2, t % 2)
            wd = wd_tasks(jnp.minimum(t * wrows, NJ * L - wrows))
            mixed = _mix(_mix(loads, wd) + sums, ln)
            side = _Tasks(mixed, sa, ska)
            gate_up_last(b, side.tick)
            for j in range(NJ - 1):
                gate_up(b, j, side.tick)
            side.flush()

        jax.lax.fori_loop(npro, nb, phase_a, None)
        mark("w", wo_copy.wait)
        side = _Tasks(mid_tasks(), 32)
        qkv(0, 0, side.tick, lambda: None)
        side.flush()
        for c in range(2 * NT):
            kv_s[c, 0:HALO, :] = jnp.broadcast_to(kv_s[c, HALO:HALO + 1, :], (HALO, L))
        jax.lax.fori_loop(0, nb - 1, lambda b, _: phase_b(b, True), None)
        phase_b(nb - 1, False)
        for b in range(nb):
            mark("e", o_copy(b).wait)

    @jax.jit
    def fn(A_x, A_wqkv, A_wo, B_x, B_w_gate, B_w_up, B_w_down):
        vm = pltpu.VMEM
        out = pl.pallas_call(
            kernel,
            in_specs=[pl.BlockSpec(memory_space=pltpu.HBM)] * 6,
            out_specs=pl.BlockSpec(memory_space=pltpu.HBM),
            out_shape=jax.ShapeDtypeStruct((S, D), A_x.dtype),
            scratch_shapes=[
                vm((nb + 1, tm, D), bf16), vm((nb + 1, 10, 2, hm, L), bf16), vm((NJ, 4 * L, D), bf16),
                vm((4, D, D), bf16), vm((2, D, D), bf16), vm((3, NJ * L, D), bf16), vm((NW * L, L), bf16), vm((NJ * 20, L, L), bf16),
                vm((NT + 1, D, L), f32), vm((2 * NT + 8, tm, L), f32), vm((4 * NT, HALO + tm, L), f32),
                vm((nb, 9, NJ, hm, L), bf16), vm((10, 2, hm, L), bf16), pltpu.SMEM((2,), jnp.int32),
                vm((nb, tm, D), A_x.dtype),
                pltpu.SemaphoreType.DMA((nb,)), pltpu.SemaphoreType.DMA((NJ,)), pltpu.SemaphoreType.DMA((6,)),
                pltpu.SemaphoreType.DMA((nb,)),
            ],
            compiler_params=pltpu.CompilerParams(vmem_limit_bytes=100 * 1024 * 1024, flags=flags),
        )(A_x.reshape(S, D), A_wqkv, A_wo, B_w_gate.T, B_w_up.T, B_w_down)
        return out.reshape(A_x.shape)

    return fn


_kernel_fn = build()


@jax.jit
def pallas_parallel_sum__sliding_local_dilated__geglu_ffn__prompt_kernel(
    A_x, A_wqkv, A_wo, B_x, B_w_gate, B_w_up, B_w_down
):
    return _kernel_fn(A_x, A_wqkv, A_wo, B_x, B_w_gate, B_w_up, B_w_down)
```

```python
import functools
import math
import jax
import jax.numpy as jnp
import jax.experimental.pallas as pl
import jax.experimental.pallas.tpu as pltpu

S, D, F = 2048, 640, 1728
H, DH, W, DIL = 32, 20, 8, 2
HALO = 16
WORDER = (0, 4, 1, 5, 2, 6, 3, 7)
L = 128
NT = D // L
NJ = 7
FM = (F // L) * L
f32, bf16, u32 = jnp.float32, jnp.bfloat16, jnp.uint32


def _dot(a, b):
    return jnp.dot(a, b, preferred_element_type=f32)


def _dot_nt(a, b):
    return jax.lax.dot_general(a, b, (((1,), (1,)), ((), ())), preferred_element_type=f32)


def _geglu(g, u):
    c = math.sqrt(2.0 / math.pi)
    t = jnp.tanh(g * (c + (c * 0.044715) * (g * g)))
    hg = 0.5 * g
    return (hg + hg * t) * u


def _lhs_terms(a11, a12, a21, a22):
    return [a11 + a22, a21 + a22, a11, a22, a11 + a12, a21 - a11, a12 - a22]


def _rhs_terms(b11, b12, b21, b22):
    return [b11 + b22, b11, b12 - b22, b21 - b11, b22, b11 + b12, b21 + b22]


ORDER = (4, 2, 3, 1, 0, 5, 6)


def _combine(m, r11, r12, r21, r22):
    return r11 - m[4] + m[3] + m[0] + m[6], r12 + m[4] + m[2], r21 + m[3] + m[1], r22 + m[2] - m[1] + m[0] + m[5]


def _put(ref, idx, r0, val, e0=0):
    n = val.shape[0]
    r = r0 if isinstance(r0, int) else pl.multiple_of(r0, n)
    for e in range(val.shape[1] // L):
        ref[idx + (e0 + e, pl.ds(r, n), slice(None))] = val[:, e * L:(e + 1) * L].astype(ref.dtype)


def _get(ref, idx, n):
    return jnp.concatenate([ref[idx + (e,)] for e in range(n)], axis=1)


def _pack(even, odd):
    return pltpu.pack_elementwise([even, odd], packed_dtype=bf16)


def _split(rows):
    words = pltpu.bitcast(rows, u32)
    return [pltpu.unpack_elementwise(words, index=i, packed_dtype=bf16, unpacked_dtype=f32) for i in range(2)]


def _grid(rows):
    return jnp.concatenate([jnp.concatenate(r, axis=1) for r in rows], axis=0)


def _mix(a, b):
    keyed = [((i + 0.5) / len(a), t) for i, t in enumerate(a)] + [((i + 0.5) / len(b), t) for i, t in enumerate(b)]
    return [t for _, t in sorted(keyed, key=lambda kt: kt[0])]


class _Tasks:
    def __init__(self, tasks, slots, skip=0):
        self.tasks, self.slots, self.skip, self.n, self.done = list(tasks), slots, skip, 0, 0

    def tick(self, val):
        for r in range(1, 5):
            self.step(val[:r * val.shape[0] // 4])

    def step(self, val):
        self.n += 0.25
        want = -(-len(self.tasks) * max(0, self.n - self.skip) // self.slots)
        while self.done < min(want, len(self.tasks)):
            self.tasks[self.done](val)
            self.done += 1

    def flush(self):
        for t in self.tasks[self.done:]:
            t(None)
        self.done = len(self.tasks)


SUMS = (0, 2, 3, 5, 6)
_GU = lambda j, n, kt, e: ((j * 5 + n) * 2 + kt) * 2 + e
_QC = lambda p, i, kt, e: ((p * 7 + i) * 2 + kt) * 2 + e
_QK = lambda p, c: _QC(4, 0, 0, 0) + p * 4 + c
_Q4 = lambda p, kt: _QK(3, 0) + p * NT + kt
_OC = lambda i, kt, e: _Q4(3, 0) + (i * 2 + kt) * 2 + e
_OK = lambda c: _OC(7, 0, 0) + c
_O4 = lambda kt: _OK(4) + kt
_DC = lambda n, e: _O4(NT) + (n * 2 + e) * NJ
NW = _DC(5, 0)


def build():
    tm, ar, lnr = 256, 16, 16
    nb = S // tm
    hm = tm // 2
    npro = 2
    wrows = 160

    def kernel(x_hbm, wqkv_hbm, wo_hbm, wg_hbm, wu_hbm, wd_hbm, o_hbm,
               x_s, xc_s, gu_r, qkv_r, wo_r, wd_r, w_s, g_s, tmp_s, a_s, q_s, kv_s, hc_s, ac_s, z_s, o_s, xsem, gsem, wsem, osem):
        def x_copy(b):
            return pltpu.make_async_copy(x_hbm.at[pl.ds(b * tm, tm)], x_s.at[b], xsem.at[b])

        def gu_copies(j):
            if j < NJ - 1:
                parts = [(wg_hbm, j * L, L, 0), (wu_hbm, j * L, L, L),
                         (wg_hbm, (j + NJ) * L, L, 2 * L), (wu_hbm, (j + NJ) * L, L, 3 * L)]
            else:
                parts = [(wg_hbm, j * L, L, 0), (wg_hbm, FM, F - FM, L), (wu_hbm, FM, F - FM, L + F - FM),
                         (wu_hbm, j * L, L, 2 * L), (wu_hbm, j * L, L, 3 * L)]
            return [pltpu.make_async_copy(src.at[pl.ds(r, n)], gu_r.at[j, pl.ds(o, n)], gsem.at[j])
                    for src, r, n, o in parts]

        def gu_wait(j):
            pltpu.make_async_copy(gu_r.at[j], gu_r.at[j], gsem.at[j]).wait()

        qkv_copies = [pltpu.make_async_copy(wqkv_hbm.at[:, pl.ds(p * D, D)], qkv_r.at[p], wsem.at[p]) for p in range(3)]
        wo_copy = pltpu.make_async_copy(wo_hbm, wo_r.at[0], wsem.at[3])
        wd_copies = [pltpu.make_async_copy(wd_hbm.at[pl.ds(0, NJ * L)], wd_r.at[0], wsem.at[4]),
                     pltpu.make_async_copy(wd_hbm.at[pl.ds(NJ * L, F - NJ * L)], wd_r.at[1, pl.ds(0, F - NJ * L)], wsem.at[5])]

        def o_copy(b):
            return pltpu.make_async_copy(o_s.at[b], o_hbm.at[pl.ds(pl.multiple_of(b * tm, tm), tm)], osem.at[b])

        def wtile(t):
            return w_s[pl.ds(t * L if isinstance(t, int) else pl.multiple_of(t * L, L), L), :]

        def set_wtile(t, val, r=0):
            n = val.shape[0]
            w_s[pl.ds(t * L + r if isinstance(t, int) else pl.multiple_of(t * L + r, n), n), :] = val.astype(bf16)

        def after(ref, spare, fn, *args):
            def task(val):
                if val is not None:
                    ref[spare + z_s[0], 0:16, 0:L] = val[-16:, -L:].astype(ref.dtype)
                fn(*args)

            return task

        def ln_tasks(b):
            dst = b
            src = b if isinstance(b, int) else jnp.minimum(b, nb - 1)

            def norm(x):
                xc = x - jnp.sum(x, axis=-1, keepdims=True) * (1.0 / D)
                v = jnp.sum(xc * xc, axis=-1, keepdims=True) * (1.0 / D)
                return xc * jax.lax.rsqrt(v + 1e-5)

            def piece(r):
                n = lnr // 2
                y = norm(jnp.concatenate(_split(x_s[src, r:r + lnr, :]) + _split(x_s[src, hm + r:hm + r + lnr, :]), axis=0))
                terms = []
                for i in range(2):
                    y1, y2 = y[i * n:(i + 1) * n], y[(2 + i) * n:(3 + i) * n]
                    terms.append(_lhs_terms(y1[:, 0:2 * L], y1[:, 2 * L:4 * L], y2[:, 0:2 * L], y2[:, 2 * L:4 * L])
                                 + [jnp.concatenate([y1[:, 4 * L:], y2[:, 4 * L:]], axis=1)])
                for i, (even, odd) in enumerate(zip(*terms)):
                    _put(xc_s, (dst, i), r // 2, _pack(even, odd))

            return [after(x_s, nb, piece, r) for r in range(0, hm, lnr)]

        def full_rows(ref, idx):
            g = lambda i, e: ref[idx + (i, e)]
            return _grid([[g(2, 0), g(2, 1), g(7, 0), g(7, 1), g(9, 0)], [g(8, 0), g(8, 1), g(3, 0), g(3, 1), g(9, 1)]])

        def project(b, wc, wk, tick):
            r = _dot_nt(pltpu.bitcast(jnp.concatenate([xc_s[b, 7, 0], xc_s[b, 7, 1]], axis=0), bf16), wk())
            tick(r)
            ms = {}
            for i in ORDER:
                ms[i] = _dot_nt(pltpu.bitcast(_get(xc_s, (b, i), 2), bf16), wc(i))
                tick(ms[i])
            n = r.shape[1] // 2
            return _combine(ms, r[:hm, :n], r[:hm, n:], r[hm:, :n], r[hm:, n:])

        def gu_tasks(j, z, ne=2):
            def piece(kt, e, r):
                t = lambda n, k: gu_r[j, (2 * n + e) * L + r:(2 * n + e) * L + r + H, k * L:(k + 1) * L].astype(f32)
                terms = _rhs_terms(t(0, kt), t(1, kt), t(0, kt + 2), t(1, kt + 2))
                for n, i in enumerate(SUMS):
                    g_s[_GU(j, n, kt, e) + z, r:r + H, :] = terms[i].astype(bf16)

            return [lambda _, a=(kt, e, r): piece(*a) for kt in range(2) for e in range(ne) for r in range(0, L, H)]

        def gu_weights(j, b22):
            def wc(i):
                if i == 1:
                    return gu_r[j, 0:2 * L, 0:2 * L]
                if i == 4:
                    return b22()
                return _grid([[g_s[_GU(j, SUMS.index(i), kt, e)] for kt in range(2)] for e in range(2)])

            return wc

        def store_h(b, j, h11, h12, h21, h22):
            for i, t in enumerate(_lhs_terms(h11, h12, h21, h22) + [h12, h21]):
                _put(hc_s, (b, i), 0, t, j)

        def gate_up(b, j, tick):
            cs = project(b, gu_weights(j, lambda: gu_r[j, 2 * L:, 2 * L:4 * L]), lambda: gu_r[j, :, 4 * L:], tick)
            store_h(b, j, *[_geglu(c[:, :L], c[:, L:]) for c in cs])

        def gate_up_last(b, tick):
            j = NJ - 1
            b22 = lambda: _grid([[gu_r[j, 2 * L:3 * L, 2 * L:4 * L]], [wtile(_Q4(2, 2)), wtile(_Q4(2, 3))]])
            wk = lambda: _grid([[gu_r[j, 0:3 * L, 4 * L:]], [wtile(_Q4(2, 4))]])
            c11, c12, c21, c22 = project(b, gu_weights(j, b22), wk, tick)
            lane = jax.lax.broadcasted_iota(jnp.int32, (hm, L), 1)
            tail = lambda t: jnp.where(lane < F - FM, _geglu(t, pltpu.roll(t, L // 2, 1)), 0.0)
            store_h(b, j, _geglu(c11[:, :L], c12[:, :L]), tail(c11[:, L:]), _geglu(c21[:, :L], c22[:, :L]), tail(c21[:, L:]))
            return c12[:, L:], c22[:, L:]

        def perm_tile(slab, c):
            return jnp.concatenate([tmp_s[slab, pl.ds(4 * c + e, H, stride=DH), :] for e in range(4)], axis=0)

        def perm_rows(slab, c, d):
            return tmp_s[slab, pl.ds(4 * c + d, H, stride=DH), :]

        def qkv_tasks(p, kt):
            def load(slab, k, c):
                rows = pl.ds(pl.multiple_of(k * L, L), L)
                tmp_s[slab, c * L:(c + 1) * L, :] = qkv_r[p, rows, c * L:(c + 1) * L].T.astype(f32)

            def sums(e, d):
                terms = _rhs_terms(perm_rows(0, e, d), perm_rows(0, 2 + e, d), perm_rows(1, e, d), perm_rows(1, 2 + e, d))
                for i, t in enumerate(terms):
                    set_wtile(_QC(p, i, kt, e), t, d * H)

            def copy(t, slab, c):
                set_wtile(t, perm_tile(slab, c))

            P = functools.partial(after, tmp_s, NT)
            return ([after(qkv_r, 3, load, s, k, c) for s, k in enumerate((kt, kt + 2, 4)) for c in range(NT)],
                    [P(copy, _Q4(p, kt), 0, 4), P(copy, _Q4(p, kt + 2), 1, 4)]
                    + [P(sums, e, d) for e in range(2) for d in range(4)]
                    + [P(copy, _Q4(p, 4), 2, 4)] + [P(copy, _QK(p, c), 2, c) for c in range(4)])

        def wd_tasks(r0):
            def piece(r, n, e):
                t = lambda k, c: wd_r[k, pl.ds(pl.multiple_of(r, 16), n), c * L:(c + 1) * L].astype(f32)
                terms = _rhs_terms(t(0, e), t(0, 2 + e), t(1, e), t(1, 2 + e))
                for m, i in enumerate(SUMS):
                    w_s[pl.ds(pl.multiple_of(_DC(m, e) * L + r, 16), n), :] = terms[i].astype(bf16)

            return [after(wd_r, 2, piece, r0 + r, H, e) for r in range(0, wrows, H) for e in range(2)]

        def mid_tasks():
            def qk4(kt, r):
                t = lambda p, k: w_s[_Q4(p, k) * L + r:_Q4(p, k) * L + r + H, :].astype(f32)
                for i, v in enumerate(_rhs_terms(t(0, kt), t(1, kt), t(0, kt + 2), t(1, kt + 2))):
                    set_wtile(_QC(3, i, kt, 0), v, r)

            def tv4(kt, r):
                t = lambda k: gu_r[NJ - 1, L + r:L + r + H, k * L:(k + 1) * L].astype(f32)
                v = lambda k: w_s[_Q4(2, k) * L + r:_Q4(2, k) * L + r + H, :].astype(f32)
                terms = _rhs_terms(t(kt), v(kt), t(kt + 2), v(kt + 2))
                for n, i in enumerate(SUMS):
                    g_s[_GU(NJ - 1, n, kt, 1), r:r + H, :] = terms[i].astype(bf16)

            def load(c, r):
                tmp_s[c, r:r + D // 2, :] = wo_r[0, r:r + D // 2, c * L:(c + 1) * L].astype(f32)

            def sums(kt, e, d):
                terms = _rhs_terms(perm_rows(e, kt, d), perm_rows(2 + e, kt, d), perm_rows(e, kt + 2, d), perm_rows(2 + e, kt + 2, d))
                for i, t in enumerate(terms):
                    set_wtile(_OC(i, kt, e), t, d * H)

            def copy(t, slab, c):
                set_wtile(t, perm_tile(slab, c))

            P = functools.partial(after, tmp_s, NT)
            for f in (tv4, qk4):
                for kt in range(2):
                    for r in range(0, L, H):
                        f(kt, r)
            stage = lambda *cs: [after(wo_r, 1, load, c, r) for c in cs for r in (0, D // 2)]
            both = lambda e: [P(sums, kt, e, d) for kt in range(2) for d in range(4)] + [P(copy, _OK(c), c, 4) for c in (e, 2 + e)]
            return stage(0, 2) + _mix(both(0), stage(1, 3)) + _mix(both(1), stage(4)) + [P(copy, _O4(kt), 4, kt) for kt in range(NT)]

        def qkv(b, tick):
            def put(p, c, r0, val):
                if p == 0:
                    q_s[b * NT + c, r0:r0 + val.shape[0], :] = val
                else:
                    kv_s[b, (p - 1) * NT + c, HALO + r0:HALO + r0 + val.shape[0], :] = val

            for p in range(3):
                wc = lambda i: _grid([[wtile(_QC(p, i, kt, e)) for kt in range(2)] for e in range(2)])
                wk = lambda: _grid([[wtile(_QK(p, c))] for c in range(4)])
                for n, cv in enumerate(project(b, wc, wk, tick)):
                    for e in range(2):
                        put(p, 2 * (n % 2) + e, hm * (n // 2), cv[:, e * L:(e + 1) * L])
            for n, cv in enumerate(gate_up_last(b, tick)):
                put(2, 4, hm * n, cv)
            wc = lambda i: _grid([[wtile(_QC(3, i, kt, 0)) for kt in range(2)]])
            wk = lambda: _grid([[wtile(_Q4(p, 4))] for p in range(2)])
            for n, cv in enumerate(project(b, wc, wk, tick)):
                put(n % 2, 4, hm * (n // 2), cv)

        def attention(b, r, out):
            q = [q_s[b * NT + c, r:r + ar, :] for c in range(NT)]
            cache = {}

            def window(slab, w):
                starts = [HALO + r - DIL * w + i for i in range(0, ar, 8)]
                for o in starts:
                    if (slab, o) not in cache:
                        cache[slab, o] = kv_s[b, slab, o:o + 8, :]
                return jnp.concatenate([cache[slab, o] for o in starts], axis=0)

            ls = []
            for w in WORDER:
                s = q[0] * window(0, w)
                for c in range(1, NT):
                    s = s + q[c] * window(c, w)
                s = (s + pltpu.roll(s, H, 1)) + (pltpu.roll(s, 2 * H, 1) + pltpu.roll(s, 3 * H, 1))
                ls.append(s)
            for n, w in enumerate(WORDER):
                if r < DIL * w:
                    row = jax.lax.broadcasted_iota(jnp.int32, (ar, L), 0) + (r + b * tm)
                    ls[n] = jnp.where(row >= DIL * w, ls[n], -1e9 * math.sqrt(DH))
            m = functools.reduce(jnp.maximum, ls)
            es = [jnp.exp2((s - m) * (math.log2(math.e) / math.sqrt(DH))) for s in ls]
            inv = 1.0 / functools.reduce(jnp.add, es)
            for c in range(NT):
                acc = None
                for n, w in enumerate(WORDER):
                    t = es[n] * window(NT + c, w)
                    acc = t if acc is None else acc + t
                out.append(acc * inv)

        def attention_pair(b, r):
            o1, o2 = [], []
            attention(b, r, o1)
            yield
            attention(b, hm + r, o2)
            for e in range(2):
                for i, t in enumerate(_lhs_terms(o1[e], o1[2 + e], o2[e], o2[2 + e]) + [o1[2 + e], o2[e], (o1, o2)[e][4]]):
                    _put(ac_s, (i,), r, t, e)

        def phase_b(b, has_next):
            if has_next:
                for c in range(2 * NT):
                    kv_s[b + 1, c, 0:HALO, :] = kv_s[b, c, tm:tm + HALO, :]
            first, slots = 2, (32 if has_next else 28)
            att = [after(q_s, nb * NT, next, g, None)
                   for g in [attention_pair(b, r) for r in range(0, hm, ar)] for _ in range(2)]
            for t in att[:first]:
                t(None)
            side = _Tasks(att[first:], slots)
            hcat = lambda i: _get(hc_s, (b, i), NJ)
            for i in ORDER:
                for e in range(2):
                    if i == 1:
                        w = wd_r[0, :, e * L:(e + 1) * L]
                    elif i == 4:
                        w = wd_r[1, :, (2 + e) * L:(3 + e) * L]
                    else:
                        w = w_s[_DC(SUMS.index(i), e) * L:(_DC(SUMS.index(i), e) + NJ) * L, :]
                    y = _dot(hcat(i), w)
                    a_s[i, e * hm:(e + 1) * hm, :] = y
                    side.tick(y[:hm // 2])
                    side.tick(y[hm // 2:])
            y = _dot(_grid([[hcat(2), hcat(7)], [hcat(8), hcat(3)]]), _grid([[wd_r[0, :, 4 * L:]], [wd_r[1, :, 4 * L:]]]))
            a_s[7] = y
            for r in range(0, tm, tm // 4):
                side.tick(y[r:r + tm // 4])
            if has_next:
                qkv(b + 1, side.tick)
            side.flush()
            r = _dot(jnp.concatenate([ac_s[9, 0], ac_s[9, 1]], axis=0), _grid([[wtile(_OK(c)) for c in range(4)]]))
            ms = {i: jnp.concatenate([a_s[i, 0:hm, :], a_s[i, hm:tm, :]], axis=1)
                  + _dot(_get(ac_s, (i,), 2), _grid([[wtile(_OC(i, kt, e)) for e in range(2)] for kt in range(2)]))
                  for i in ORDER}
            quads = [(slice(hm * m, hm * (m + 1)), slice(2 * L * n, 2 * L * (n + 1))) for m in range(2) for n in range(2)]
            for (rs, cl), cv in zip(quads, _combine(ms, *[x_s[b, rs, cl].astype(f32) + r[rs, cl] for rs, cl in quads])):
                o_s[b, rs, cl] = cv.astype(o_s.dtype)
            y4 = a_s[7] + _dot(full_rows(ac_s, ()), w_s[_O4(0) * L:_O4(NT) * L, :])
            o_s[b, :, 4 * L:] = (x_s[b, :, 4 * L:].astype(f32) + y4).astype(o_s.dtype)
            o_copy(b).start()

        def start(copies):
            for cp in copies:
                cp.start()

        start([x_copy(0)] + gu_copies(0) + [x_copy(1)])
        z_s[0] = 0
        wd_r[1, F - NJ * L:, :] = jnp.zeros((2 * NJ * L - F, D), bf16)
        x_copy(0).wait()
        start(gu_copies(1))
        _Tasks(ln_tasks(0), 1).flush()
        gu_wait(0)
        start(gu_copies(2))
        _Tasks(gu_tasks(0, 0), 1).flush()
        later = [gu_copies(3) + gu_copies(4), gu_copies(5) + gu_copies(6) + [x_copy(2), x_copy(3)],
                 qkv_copies[:1] + wd_copies[:1], wd_copies[1:], [x_copy(4)] + qkv_copies[1:], [wo_copy]]

        def run(tasks, slots, blocks, j):
            side = _Tasks(tasks, slots)
            for b in blocks:
                gate_up(b, j, side.tick)
            side.flush()

        def prologue(j, _):
            gu_wait(j + 1)
            for n in range(1, NJ - 2):
                pl.when(j == n)(functools.partial(start, later[n]))
            run(gu_tasks(j + 1, z_s[0]), 14, (0, 1), j)

        x_copy(1).wait()
        run(ln_tasks(1), 6, (0,), 0)
        gu_wait(1)
        start(later[0])
        run(gu_tasks(1, z_s[0]), 7, (1,), 0)
        jax.lax.fori_loop(1, NJ - 2, prologue, None)
        gu_wait(NJ - 1)
        x_copy(npro).wait()
        start(later[NJ - 2])
        run(_mix(ln_tasks(npro), gu_tasks(NJ - 1, z_s[0], 1)), 13, (0, 1), NJ - 2)
        start([x_copy(b) for b in range(5, nb)])
        qkv_copies[0].wait()
        for cp in wd_copies:
            cp.wait()

        def phase_a(b, _):
            t = b - npro
            pl.when(b + 1 < nb)(lambda: x_copy(b + 1).wait())
            for p in (1, 2):
                pl.when(t == 2 * p)(qkv_copies[p].wait)
            ln = ln_tasks(b + 1)
            loads, sums = qkv_tasks(t // 2, t % 2)
            wd = wd_tasks(jnp.minimum(t * wrows, NJ * L - wrows))
            mixed = _mix(_mix(loads, wd) + sums, ln)
            side = _Tasks(mixed, 45)
            for j in range(NJ - 1):
                gate_up(b, j, side.tick)
            side.flush()

        jax.lax.fori_loop(npro, nb, phase_a, None)
        wo_copy.wait()
        side = _Tasks(mid_tasks(), 32, 2)
        qkv(0, side.tick)
        side.flush()
        for c in range(2 * NT):
            kv_s[0, c, 0:HALO, :] = jnp.broadcast_to(kv_s[0, c, HALO:HALO + 1, :], (HALO, L))
        jax.lax.fori_loop(0, nb - 1, lambda b, _: phase_b(b, True), None)
        phase_b(nb - 1, False)
        for b in range(nb):
            o_copy(b).wait()

    def fn(A_x, A_wqkv, A_wo, B_x, B_w_gate, B_w_up, B_w_down):
        vm = pltpu.VMEM
        out = pl.pallas_call(
            kernel,
            in_specs=[pl.BlockSpec(memory_space=pltpu.HBM)] * 6,
            out_specs=pl.BlockSpec(memory_space=pltpu.HBM),
            out_shape=jax.ShapeDtypeStruct((S, D), A_x.dtype),
            scratch_shapes=[
                vm((nb + 1, tm, D), bf16), vm((nb + 1, 8, 2, hm // 2, L), u32), vm((NJ, 4 * L, D), bf16),
                vm((4, D, D), bf16), vm((2, D, D), bf16), vm((3, NJ * L, D), bf16), vm((NW * L, L), bf16), vm((NJ * 20, L, L), bf16),
                vm((NT + 1, D, L), f32), vm((8, tm, L), f32), vm((nb * NT + 1, tm, L), f32), vm((nb, 2 * NT, HALO + tm, L), f32),
                vm((nb, 9, NJ, hm, L), bf16), vm((10, 2, hm, L), bf16), pltpu.SMEM((2,), jnp.int32),
                vm((nb, tm, D), A_x.dtype),
                pltpu.SemaphoreType.DMA((nb,)), pltpu.SemaphoreType.DMA((NJ,)), pltpu.SemaphoreType.DMA((6,)),
                pltpu.SemaphoreType.DMA((nb,)),
            ],
            compiler_params=pltpu.CompilerParams(vmem_limit_bytes=100 * 1024 * 1024),
        )(A_x.reshape(S, D), A_wqkv, A_wo, B_w_gate.T, B_w_up.T, B_w_down)
        return out.reshape(A_x.shape)

    return fn


@jax.jit
def pallas_parallel_sum__sliding_local_dilated__geglu_ffn__prompt_kernel(
    A_x, A_wqkv, A_wo, B_x, B_w_gate, B_w_up, B_w_down
):
    return build()(A_x, A_wqkv, A_wo, B_x, B_w_gate, B_w_up, B_w_down)
```

```python
import functools
import math
import jax
import jax.numpy as jnp
import jax.experimental.pallas as pl
import jax.experimental.pallas.tpu as pltpu

S, D, F = 2048, 640, 1728
H, DH, W, DIL = 32, 20, 8, 2
HALO = 16
WORDER = (0, 4, 1, 5, 2, 6, 3, 7)
L = 128
NT = D // L
NJ = 7
FM = (F // L) * L
f32, bf16 = jnp.float32, jnp.bfloat16


def _dot(a, b):
    return jnp.dot(a, b, preferred_element_type=f32)


def _dot_nt(a, b):
    return jax.lax.dot_general(a, b, (((1,), (1,)), ((), ())), preferred_element_type=f32)


def _geglu(g, u):
    c = math.sqrt(2.0 / math.pi)
    t = jnp.tanh(g * (c + (c * 0.044715) * (g * g)))
    hg = 0.5 * g
    return (hg + hg * t) * u


def _lhs_terms(a11, a12, a21, a22):
    return [a11 + a22, a21 + a22, a11, a22, a11 + a12, a21 - a11, a12 - a22]


def _rhs_terms(b11, b12, b21, b22):
    return [b11 + b22, b11, b12 - b22, b21 - b11, b22, b11 + b12, b21 + b22]


ORDER = (4, 2, 3, 1, 0, 5, 6)


def _combine(m, r11, r12, r21, r22):
    return r11 - m[4] + m[3] + m[0] + m[6], r12 + m[4] + m[2], r21 + m[3] + m[1], r22 + m[2] - m[1] + m[0] + m[5]


def _put(ref, idx, r0, val, e0=0):
    n = val.shape[0]
    r = r0 if isinstance(r0, int) else pl.multiple_of(r0, n)
    for e in range(val.shape[1] // L):
        ref[idx + (e0 + e, pl.ds(r, n), slice(None))] = val[:, e * L:(e + 1) * L].astype(ref.dtype)


def _get(ref, idx, n):
    return jnp.concatenate([ref[idx + (e,)] for e in range(n)], axis=1)


def _grid(rows):
    return jnp.concatenate([jnp.concatenate(r, axis=1) for r in rows], axis=0)


def _mix(a, b):
    keyed = [((i + 0.5) / len(a), t) for i, t in enumerate(a)] + [((i + 0.5) / len(b), t) for i, t in enumerate(b)]
    return [t for _, t in sorted(keyed, key=lambda kt: kt[0])]


class _Tasks:
    def __init__(self, tasks, slots, skip=0):
        self.tasks, self.slots, self.skip, self.n, self.done = list(tasks), slots, skip, 0, 0

    def tick(self, val):
        for r in range(1, 5):
            self.step(val[:r * val.shape[0] // 4])

    def step(self, val):
        self.n += 0.25
        want = -(-len(self.tasks) * max(0, self.n - self.skip) // self.slots)
        while self.done < min(want, len(self.tasks)):
            self.tasks[self.done](val)
            self.done += 1

    def flush(self):
        for t in self.tasks[self.done:]:
            t(None)
        self.done = len(self.tasks)


SUMS = (0, 2, 3, 5, 6)
_GU = lambda j, n, kt, e: ((j * 5 + n) * 2 + kt) * 2 + e
_QC = lambda p, i, kt, e: ((p * 7 + i) * 2 + kt) * 2 + e
_QK = lambda p, c: _QC(4, 0, 0, 0) + p * 4 + c
_Q4 = lambda p, kt: _QK(3, 0) + p * NT + kt
_OC = lambda i, kt, e: _Q4(3, 0) + (i * 2 + kt) * 2 + e
_OK = lambda c: _OC(7, 0, 0) + c
_O4 = lambda kt: _OK(4) + kt
_DC = lambda n, e: _O4(NT) + (n * 2 + e) * NJ
NW = _DC(5, 0)


def build():
    tm, ar, lnr = 256, 16, 16
    nb = S // tm
    hm = tm // 2
    npro = 2
    wrows = 160

    def kernel(x_hbm, wqkv_hbm, wo_hbm, wg_hbm, wu_hbm, wd_hbm, o_hbm,
               x_s, xc_s, gu_r, qkv_r, wo_r, wd_r, w_s, g_s, tmp_s, a_s, q_s, kv_s, hc_s, ac_s, z_s, o_s, xsem, gsem, wsem, osem):
        def x_copy(b):
            return pltpu.make_async_copy(x_hbm.at[pl.ds(b * tm, tm)], x_s.at[b], xsem.at[b])

        def gu_copies(j):
            if j < NJ - 1:
                parts = [(wg_hbm, j * L, L, 0), (wu_hbm, j * L, L, L),
                         (wg_hbm, (j + NJ) * L, L, 2 * L), (wu_hbm, (j + NJ) * L, L, 3 * L)]
            else:
                parts = [(wg_hbm, j * L, L, 0), (wg_hbm, FM, F - FM, L), (wu_hbm, FM, F - FM, L + F - FM),
                         (wu_hbm, j * L, L, 2 * L), (wu_hbm, j * L, L, 3 * L)]
            return [pltpu.make_async_copy(src.at[pl.ds(r, n)], gu_r.at[j, pl.ds(o, n)], gsem.at[j])
                    for src, r, n, o in parts]

        def gu_wait(j):
            pltpu.make_async_copy(gu_r.at[j], gu_r.at[j], gsem.at[j]).wait()

        qkv_copies = [pltpu.make_async_copy(wqkv_hbm.at[:, pl.ds(p * D, D)], qkv_r.at[p], wsem.at[p]) for p in range(3)]
        wo_copy = pltpu.make_async_copy(wo_hbm, wo_r.at[0], wsem.at[3])
        wd_copies = [pltpu.make_async_copy(wd_hbm.at[pl.ds(0, NJ * L)], wd_r.at[0], wsem.at[4]),
                     pltpu.make_async_copy(wd_hbm.at[pl.ds(NJ * L, F - NJ * L)], wd_r.at[1, pl.ds(0, F - NJ * L)], wsem.at[5])]

        def o_copy(b):
            return pltpu.make_async_copy(o_s.at[b], o_hbm.at[pl.ds(pl.multiple_of(b * tm, tm), tm)], osem.at[b])

        def wtile(t):
            return w_s[pl.ds(t * L if isinstance(t, int) else pl.multiple_of(t * L, L), L), :]

        def set_wtile(t, val, r=0):
            n = val.shape[0]
            w_s[pl.ds(t * L + r if isinstance(t, int) else pl.multiple_of(t * L + r, n), n), :] = val.astype(bf16)

        def after(ref, spare, fn, *args):
            def task(val):
                if val is not None:
                    ref[spare + z_s[0], 0:16, 0:L] = val[-16:, -L:].astype(ref.dtype)
                fn(*args)

            return task

        def ln_tasks(b):
            dst = b
            src = b if isinstance(b, int) else jnp.minimum(b, nb - 1)

            def norm(x):
                xc = x - jnp.sum(x, axis=-1, keepdims=True) * (1.0 / D)
                v = jnp.sum(xc * xc, axis=-1, keepdims=True) * (1.0 / D)
                return xc * jax.lax.rsqrt(v + 1e-5)

            def piece(r):
                y = norm(jnp.concatenate([x_s[src, m + r:m + r + lnr, :].astype(f32) for m in (0, hm)], axis=0))
                y1, y2 = y[:lnr], y[lnr:]
                terms = _lhs_terms(y1[:, 0:2 * L], y1[:, 2 * L:4 * L], y2[:, 0:2 * L], y2[:, 2 * L:4 * L])
                for i, t in enumerate(terms + [jnp.concatenate([y1[:, 4 * L:], y2[:, 4 * L:]], axis=1)]):
                    _put(xc_s, (dst, i), r, t)

            return [after(x_s, nb, piece, r) for r in range(0, hm, lnr)]

        def full_rows(ref, idx):
            g = lambda i, e: ref[idx + (i, e)]
            return _grid([[g(2, 0), g(2, 1), g(7, 0), g(7, 1), g(9, 0)], [g(8, 0), g(8, 1), g(3, 0), g(3, 1), g(9, 1)]])

        def project(b, wc, wk, tick):
            r = _dot_nt(jnp.concatenate([xc_s[b, 7, 0], xc_s[b, 7, 1]], axis=0), wk())
            tick(r)
            ms = {}
            for i in ORDER:
                ms[i] = _dot_nt(_get(xc_s, (b, i), 2), wc(i))
                tick(ms[i])
            n = r.shape[1] // 2
            return _combine(ms, r[:hm, :n], r[:hm, n:], r[hm:, :n], r[hm:, n:])

        def gu_tasks(j, z, ne=2):
            def piece(kt, e, r):
                t = lambda n, k: gu_r[j, (2 * n + e) * L + r:(2 * n + e) * L + r + H, k * L:(k + 1) * L].astype(f32)
                terms = _rhs_terms(t(0, kt), t(1, kt), t(0, kt + 2), t(1, kt + 2))
                for n, i in enumerate(SUMS):
                    g_s[_GU(j, n, kt, e) + z, r:r + H, :] = terms[i].astype(bf16)

            return [lambda _, a=(kt, e, r): piece(*a) for kt in range(2) for e in range(ne) for r in range(0, L, H)]

        def gu_weights(j, b22):
            def wc(i):
                if i == 1:
                    return gu_r[j, 0:2 * L, 0:2 * L]
                if i == 4:
                    return b22()
                return _grid([[g_s[_GU(j, SUMS.index(i), kt, e)] for kt in range(2)] for e in range(2)])

            return wc

        def store_h(b, j, h11, h12, h21, h22):
            for i, t in enumerate(_lhs_terms(h11, h12, h21, h22) + [h12, h21]):
                _put(hc_s, (b, i), 0, t, j)

        def gate_up(b, j, tick):
            cs = project(b, gu_weights(j, lambda: gu_r[j, 2 * L:, 2 * L:4 * L]), lambda: gu_r[j, :, 4 * L:], tick)
            store_h(b, j, *[_geglu(c[:, :L], c[:, L:]) for c in cs])

        def gate_up_last(b, tick):
            j = NJ - 1
            b22 = lambda: _grid([[gu_r[j, 2 * L:3 * L, 2 * L:4 * L]], [wtile(_Q4(2, 2)), wtile(_Q4(2, 3))]])
            wk = lambda: _grid([[gu_r[j, 0:3 * L, 4 * L:]], [wtile(_Q4(2, 4))]])
            c11, c12, c21, c22 = project(b, gu_weights(j, b22), wk, tick)
            lane = jax.lax.broadcasted_iota(jnp.int32, (hm, L), 1)
            tail = lambda t: jnp.where(lane < F - FM, _geglu(t, pltpu.roll(t, L // 2, 1)), 0.0)
            store_h(b, j, _geglu(c11[:, :L], c12[:, :L]), tail(c11[:, L:]), _geglu(c21[:, :L], c22[:, :L]), tail(c21[:, L:]))
            return c12[:, L:], c22[:, L:]

        def perm_tile(slab, c):
            return jnp.concatenate([tmp_s[slab, pl.ds(4 * c + e, H, stride=DH), :] for e in range(4)], axis=0)

        def perm_rows(slab, c, d):
            return tmp_s[slab, pl.ds(4 * c + d, H, stride=DH), :]

        def qkv_tasks(p, kt):
            def load(slab, k, c):
                rows = pl.ds(pl.multiple_of(k * L, L), L)
                tmp_s[slab, c * L:(c + 1) * L, :] = qkv_r[p, rows, c * L:(c + 1) * L].T.astype(f32)

            def sums(e, d):
                terms = _rhs_terms(perm_rows(0, e, d), perm_rows(0, 2 + e, d), perm_rows(1, e, d), perm_rows(1, 2 + e, d))
                for i, t in enumerate(terms):
                    set_wtile(_QC(p, i, kt, e), t, d * H)

            def copy(t, slab, c):
                set_wtile(t, perm_tile(slab, c))

            P = functools.partial(after, tmp_s, NT)
            return ([after(qkv_r, 3, load, s, k, c) for s, k in enumerate((kt, kt + 2, 4)) for c in range(NT)],
                    [P(copy, _Q4(p, kt), 0, 4), P(copy, _Q4(p, kt + 2), 1, 4)]
                    + [P(sums, e, d) for e in range(2) for d in range(4)]
                    + [P(copy, _Q4(p, 4), 2, 4)] + [P(copy, _QK(p, c), 2, c) for c in range(4)])

        def wd_tasks(r0):
            def piece(r, n, e):
                t = lambda k, c: wd_r[k, pl.ds(pl.multiple_of(r, 16), n), c * L:(c + 1) * L].astype(f32)
                terms = _rhs_terms(t(0, e), t(0, 2 + e), t(1, e), t(1, 2 + e))
                for m, i in enumerate(SUMS):
                    w_s[pl.ds(pl.multiple_of(_DC(m, e) * L + r, 16), n), :] = terms[i].astype(bf16)

            return [after(wd_r, 2, piece, r0 + r, H, e) for r in range(0, wrows, H) for e in range(2)]

        def mid_tasks():
            def qk4(kt, r):
                t = lambda p, k: w_s[_Q4(p, k) * L + r:_Q4(p, k) * L + r + H, :].astype(f32)
                for i, v in enumerate(_rhs_terms(t(0, kt), t(1, kt), t(0, kt + 2), t(1, kt + 2))):
                    set_wtile(_QC(3, i, kt, 0), v, r)

            def tv4(kt, r):
                t = lambda k: gu_r[NJ - 1, L + r:L + r + H, k * L:(k + 1) * L].astype(f32)
                v = lambda k: w_s[_Q4(2, k) * L + r:_Q4(2, k) * L + r + H, :].astype(f32)
                terms = _rhs_terms(t(kt), v(kt), t(kt + 2), v(kt + 2))
                for n, i in enumerate(SUMS):
                    g_s[_GU(NJ - 1, n, kt, 1), r:r + H, :] = terms[i].astype(bf16)

            def load(c, r):
                tmp_s[c, r:r + D // 2, :] = wo_r[0, r:r + D // 2, c * L:(c + 1) * L].astype(f32)

            def sums(kt, e, d):
                terms = _rhs_terms(perm_rows(e, kt, d), perm_rows(2 + e, kt, d), perm_rows(e, kt + 2, d), perm_rows(2 + e, kt + 2, d))
                for i, t in enumerate(terms):
                    set_wtile(_OC(i, kt, e), t, d * H)

            def copy(t, slab, c):
                set_wtile(t, perm_tile(slab, c))

            P = functools.partial(after, tmp_s, NT)
            for f in (tv4, qk4):
                for kt in range(2):
                    for r in range(0, L, H):
                        f(kt, r)
            stage = lambda *cs: [after(wo_r, 1, load, c, r) for c in cs for r in (0, D // 2)]
            both = lambda e: [P(sums, kt, e, d) for kt in range(2) for d in range(4)] + [P(copy, _OK(c), c, 4) for c in (e, 2 + e)]
            return stage(0, 2) + _mix(both(0), stage(1, 3)) + _mix(both(1), stage(4)) + [P(copy, _O4(kt), 4, kt) for kt in range(NT)]

        def qkv(b, tick):
            def put(p, c, r0, val):
                if p == 0:
                    q_s[b * NT + c, r0:r0 + val.shape[0], :] = val
                else:
                    kv_s[b, (p - 1) * NT + c, HALO + r0:HALO + r0 + val.shape[0], :] = val

            for p in range(3):
                wc = lambda i: _grid([[wtile(_QC(p, i, kt, e)) for kt in range(2)] for e in range(2)])
                wk = lambda: _grid([[wtile(_QK(p, c))] for c in range(4)])
                for n, cv in enumerate(project(b, wc, wk, tick)):
                    for e in range(2):
                        put(p, 2 * (n % 2) + e, hm * (n // 2), cv[:, e * L:(e + 1) * L])
            for n, cv in enumerate(gate_up_last(b, tick)):
                put(2, 4, hm * n, cv)
            wc = lambda i: _grid([[wtile(_QC(3, i, kt, 0)) for kt in range(2)]])
            wk = lambda: _grid([[wtile(_Q4(p, 4))] for p in range(2)])
            for n, cv in enumerate(project(b, wc, wk, tick)):
                put(n % 2, 4, hm * (n // 2), cv)

        def attention(b, r, out):
            q = [q_s[b * NT + c, r:r + ar, :] for c in range(NT)]
            cache = {}

            def window(slab, w):
                starts = [HALO + r - DIL * w + i for i in range(0, ar, 8)]
                for o in starts:
                    if (slab, o) not in cache:
                        cache[slab, o] = kv_s[b, slab, o:o + 8, :]
                return jnp.concatenate([cache[slab, o] for o in starts], axis=0)

            ls = []
            for w in WORDER:
                s = q[0] * window(0, w)
                for c in range(1, NT):
                    s = s + q[c] * window(c, w)
                s = (s + pltpu.roll(s, H, 1)) + (pltpu.roll(s, 2 * H, 1) + pltpu.roll(s, 3 * H, 1))
                ls.append(s)
            for n, w in enumerate(WORDER):
                if r < DIL * w:
                    row = jax.lax.broadcasted_iota(jnp.int32, (ar, L), 0) + (r + b * tm)
                    ls[n] = jnp.where(row >= DIL * w, ls[n], -1e9 * math.sqrt(DH))
            m = functools.reduce(jnp.maximum, ls)
            es = [jnp.exp2((s - m) * (math.log2(math.e) / math.sqrt(DH))) for s in ls]
            inv = 1.0 / functools.reduce(jnp.add, es)
            for c in range(NT):
                acc = None
                for n, w in enumerate(WORDER):
                    t = es[n] * window(NT + c, w)
                    acc = t if acc is None else acc + t
                out.append(acc * inv)

        def attention_pair(b, r):
            o1, o2 = [], []
            attention(b, r, o1)
            yield
            attention(b, hm + r, o2)
            for e in range(2):
                for i, t in enumerate(_lhs_terms(o1[e], o1[2 + e], o2[e], o2[2 + e]) + [o1[2 + e], o2[e], (o1, o2)[e][4]]):
                    _put(ac_s, (i,), r, t, e)

        def phase_b(b, has_next):
            if has_next:
                for c in range(2 * NT):
                    kv_s[b + 1, c, 0:HALO, :] = kv_s[b, c, tm:tm + HALO, :]
            first, slots = 2, (32 if has_next else 28)
            att = [after(q_s, nb * NT, next, g, None)
                   for g in [attention_pair(b, r) for r in range(0, hm, ar)] for _ in range(2)]
            for t in att[:first]:
                t(None)
            side = _Tasks(att[first:], slots)
            hcat = lambda i: _get(hc_s, (b, i), NJ)
            for i in ORDER:
                for e in range(2):
                    if i == 1:
                        w = wd_r[0, :, e * L:(e + 1) * L]
                    elif i == 4:
                        w = wd_r[1, :, (2 + e) * L:(3 + e) * L]
                    else:
                        w = w_s[_DC(SUMS.index(i), e) * L:(_DC(SUMS.index(i), e) + NJ) * L, :]
                    y = _dot(hcat(i), w)
                    a_s[i, e * hm:(e + 1) * hm, :] = y
                    side.tick(y[:hm // 2])
                    side.tick(y[hm // 2:])
            y = _dot(_grid([[hcat(2), hcat(7)], [hcat(8), hcat(3)]]), _grid([[wd_r[0, :, 4 * L:]], [wd_r[1, :, 4 * L:]]]))
            a_s[7] = y
            for r in range(0, tm, tm // 4):
                side.tick(y[r:r + tm // 4])
            if has_next:
                qkv(b + 1, side.tick)
            side.flush()
            r = _dot(jnp.concatenate([ac_s[9, 0], ac_s[9, 1]], axis=0), _grid([[wtile(_OK(c)) for c in range(4)]]))
            ms = {i: jnp.concatenate([a_s[i, 0:hm, :], a_s[i, hm:tm, :]], axis=1)
                  + _dot(_get(ac_s, (i,), 2), _grid([[wtile(_OC(i, kt, e)) for e in range(2)] for kt in range(2)]))
                  for i in ORDER}
            quads = [(slice(hm * m, hm * (m + 1)), slice(2 * L * n, 2 * L * (n + 1))) for m in range(2) for n in range(2)]
            for (rs, cl), cv in zip(quads, _combine(ms, *[x_s[b, rs, cl].astype(f32) + r[rs, cl] for rs, cl in quads])):
                o_s[b, rs, cl] = cv.astype(o_s.dtype)
            y4 = a_s[7] + _dot(full_rows(ac_s, ()), w_s[_O4(0) * L:_O4(NT) * L, :])
            o_s[b, :, 4 * L:] = (x_s[b, :, 4 * L:].astype(f32) + y4).astype(o_s.dtype)
            o_copy(b).start()

        def start(copies):
            for cp in copies:
                cp.start()

        start([x_copy(0)] + gu_copies(0) + [x_copy(1)])
        z_s[0] = 0
        wd_r[1, F - NJ * L:, :] = jnp.zeros((2 * NJ * L - F, D), bf16)
        x_copy(0).wait()
        start(gu_copies(1))
        _Tasks(ln_tasks(0), 1).flush()
        gu_wait(0)
        start(gu_copies(2))
        _Tasks(gu_tasks(0, 0), 1).flush()
        later = [gu_copies(3) + gu_copies(4), gu_copies(5) + gu_copies(6) + [x_copy(2), x_copy(3)],
                 qkv_copies[:1] + wd_copies[:1], wd_copies[1:], [x_copy(4)] + qkv_copies[1:], [wo_copy]]

        def run(tasks, slots, blocks, j):
            side = _Tasks(tasks, slots)
            for b in blocks:
                gate_up(b, j, side.tick)
            side.flush()

        def prologue(j, _):
            gu_wait(j + 1)
            for n in range(1, NJ - 2):
                pl.when(j == n)(functools.partial(start, later[n]))
            run(gu_tasks(j + 1, z_s[0]), 14, (0, 1), j)

        x_copy(1).wait()
        run(ln_tasks(1), 6, (0,), 0)
        gu_wait(1)
        start(later[0])
        run(gu_tasks(1, z_s[0]), 7, (1,), 0)
        jax.lax.fori_loop(1, NJ - 2, prologue, None)
        gu_wait(NJ - 1)
        x_copy(npro).wait()
        start(later[NJ - 2])
        run(_mix(ln_tasks(npro), gu_tasks(NJ - 1, z_s[0], 1)), 13, (0, 1), NJ - 2)
        start([x_copy(b) for b in range(5, nb)])
        qkv_copies[0].wait()
        for cp in wd_copies:
            cp.wait()

        def phase_a(b, _):
            t = b - npro
            pl.when(b + 1 < nb)(lambda: x_copy(b + 1).wait())
            for p in (1, 2):
                pl.when(t == 2 * p)(qkv_copies[p].wait)
            ln = ln_tasks(b + 1)
            loads, sums = qkv_tasks(t // 2, t % 2)
            wd = wd_tasks(jnp.minimum(t * wrows, NJ * L - wrows))
            mixed = _mix(_mix(loads, wd) + sums, ln)
            side = _Tasks(mixed, 45)
            for j in range(NJ - 1):
                gate_up(b, j, side.tick)
            side.flush()

        jax.lax.fori_loop(npro, nb, phase_a, None)
        wo_copy.wait()
        side = _Tasks(mid_tasks(), 32, 2)
        qkv(0, side.tick)
        side.flush()
        for c in range(2 * NT):
            kv_s[0, c, 0:HALO, :] = jnp.broadcast_to(kv_s[0, c, HALO:HALO + 1, :], (HALO, L))
        jax.lax.fori_loop(0, nb - 1, lambda b, _: phase_b(b, True), None)
        phase_b(nb - 1, False)
        for b in range(nb):
            o_copy(b).wait()

    def fn(A_x, A_wqkv, A_wo, B_x, B_w_gate, B_w_up, B_w_down):
        vm = pltpu.VMEM
        out = pl.pallas_call(
            kernel,
            in_specs=[pl.BlockSpec(memory_space=pltpu.HBM)] * 6,
            out_specs=pl.BlockSpec(memory_space=pltpu.HBM),
            out_shape=jax.ShapeDtypeStruct((S, D), A_x.dtype),
            scratch_shapes=[
                vm((nb + 1, tm, D), bf16), vm((nb + 1, 8, 2, hm, L), bf16), vm((NJ, 4 * L, D), bf16),
                vm((4, D, D), bf16), vm((2, D, D), bf16), vm((3, NJ * L, D), bf16), vm((NW * L, L), bf16), vm((NJ * 20, L, L), bf16),
                vm((NT + 1, D, L), f32), vm((8, tm, L), f32), vm((nb * NT + 1, tm, L), f32), vm((nb, 2 * NT, HALO + tm, L), f32),
                vm((nb, 9, NJ, hm, L), bf16), vm((10, 2, hm, L), bf16), pltpu.SMEM((2,), jnp.int32),
                vm((nb, tm, D), A_x.dtype),
                pltpu.SemaphoreType.DMA((nb,)), pltpu.SemaphoreType.DMA((NJ,)), pltpu.SemaphoreType.DMA((6,)),
                pltpu.SemaphoreType.DMA((nb,)),
            ],
            compiler_params=pltpu.CompilerParams(vmem_limit_bytes=100 * 1024 * 1024),
        )(A_x.reshape(S, D), A_wqkv, A_wo, B_w_gate.T, B_w_up.T, B_w_down)
        return out.reshape(A_x.shape)

    return fn


@jax.jit
def pallas_parallel_sum__sliding_local_dilated__geglu_ffn__prompt_kernel(
    A_x, A_wqkv, A_wo, B_x, B_w_gate, B_w_up, B_w_down
):
    return build()(A_x, A_wqkv, A_wo, B_x, B_w_gate, B_w_up, B_w_down)
```
